```python
import os as _os
_os.environ.setdefault("JAX_PLATFORMS", "cpu")
import jax
import jax.numpy as jnp

def _softmax(x, axis=-1):
    return jax.nn.softmax(x, axis=axis)
def _gelu(x):
    return jax.nn.gelu(x, approximate=True)
def _silu(x):
    return jax.nn.silu(x)
def _sigmoid(x):
    return jax.nn.sigmoid(x)
def _layernorm(x, axis=-1, eps=1e-5):
    m = jnp.mean(x, axis=axis, keepdims=True)
    v = jnp.var(x, axis=axis, keepdims=True)
    return (x - m) / jnp.sqrt(v + eps)
def _scatter_add(tgt, idx, src, axis=0):
    return tgt.at[idx].add(src)
def _segment_sum(src, seg, n):
    return jax.ops.segment_sum(src, seg, n)
class _Rng:
    def __init__(self, key):
        self._k = key
    def _next(self):
        self._k, sub = jax.random.split(self._k)
        return sub
    def normal(self, shape):
        return jax.random.normal(self._next(), shape, dtype=jnp.bfloat16)
    def randint(self, lo, hi, shape):
        return jax.random.randint(self._next(), shape, lo, hi, dtype=jnp.int32)
    def uniform(self, shape, lo=0.0, hi=1.0):
        return jax.random.uniform(self._next(), shape, jnp.bfloat16, lo, hi)
    def permutation(self, n):
        return jax.random.permutation(self._next(), n)


kernel_name = 'standalone__mha_block_cached__near_ridge'

def setup_inputs():
    _rng = _Rng(jax.random.key(int.from_bytes(__import__("os").urandom(4), "little")))
    _w = (lambda a: (lambda t: t.astype(jnp.bfloat16) if jnp.issubdtype(t.dtype, jnp.floating) else t)(jnp.asarray(a)))
    B, Sq, D = 8, 144, 448
    H, Sk, Dh = 16, 2048, 256
    return {
        "x": _w((lambda *s: _rng.normal(s) * 0.8)(B, Sq, D)),
        "k_cache": _w((lambda *s: _rng.normal(s) * 0.8)(B, H, Sk, Dh)),
        "v_cache": _w((lambda *s: _rng.normal(s) * 0.05)(B, H, Sk, Dh)),
        "wq": _w((lambda *s: _rng.normal(s) * 0.8)(D, H * Dh) * (D ** -0.5)),
        "wo": _w((lambda *s: _rng.normal(s) * 0.05)(H * Dh, D) * ((H * Dh) ** -0.5)),
    }

def reference(x, k_cache, v_cache, wq, wo):
    B, Sq, D = x.shape
    H, Dh = 16, 256
    q = (lambda x, *d: x.transpose(*d))((x @ wq).reshape(B, Sq, H, Dh), 0, 2, 1, 3)
    scores = jnp.einsum("bhqd,bhkd->bhqk", q, k_cache) * (Dh ** -0.5)
    p = _softmax(scores, axis=-1)
    o = jnp.einsum("bhqk,bhkd->bhqd", p, v_cache)
    return (lambda x, *d: x.transpose(*d))(o, 0, 2, 1, 3).reshape(B, Sq, H * Dh) @ wo
```

```python
import jax
import jax.numpy as jnp
from jax import lax
import jax.experimental.pallas as pl
import jax.experimental.pallas.tpu as pltpu


@jax.jit
def pallas_standalone__mha_block_cached__near_ridge_kernel(
    x: jax.Array,
    k_cache: jax.Array,
    v_cache: jax.Array,
    wq: jax.Array,
    wo: jax.Array,
):
    B, Sq, D = x.shape
    _, H, Sk, Dh = k_cache.shape
    scale = Dh ** -0.5
    nt = (((1,), (1,)), ((), ()))

    def kern(x_ref, k_ref, v_ref, wq_ref, wot_ref, o_ref, acc_ref):
        h = pl.program_id(1)
        col = pl.multiple_of(h * Dh, Dh)

        @pl.when(h == 0)
        def _():
            acc_ref[...] = jnp.zeros_like(acc_ref)

        q = jnp.dot(x_ref[0], wq_ref[:, pl.ds(col, Dh)], preferred_element_type=jnp.float32)
        q = (q * scale).astype(jnp.bfloat16)
        s = lax.dot_general(q, k_ref[0, 0], nt, preferred_element_type=jnp.float32)
        m = jnp.max(s, axis=-1, keepdims=True)
        p = jnp.exp(s - m)
        l = jnp.sum(p, axis=-1, keepdims=True)
        o = jnp.dot(p.astype(jnp.bfloat16), v_ref[0, 0], preferred_element_type=jnp.float32)
        o = (o / l).astype(jnp.bfloat16)
        acc_ref[...] += lax.dot_general(o, wot_ref[:, pl.ds(col, Dh)], nt,
                                        preferred_element_type=jnp.float32)

        @pl.when(h == pl.num_programs(1) - 1)
        def _():
            o_ref[0] = acc_ref[...].astype(o_ref.dtype)

    return pl.pallas_call(
        kern,
        grid=(B, H),
        in_specs=[
            pl.BlockSpec((1, Sq, D), lambda b, h: (b, 0, 0)),
            pl.BlockSpec((1, 1, Sk, Dh), lambda b, h: (b, h, 0, 0)),
            pl.BlockSpec((1, 1, Sk, Dh), lambda b, h: (b, h, 0, 0)),
            pl.BlockSpec((D, H * Dh), lambda b, h: (0, 0)),
            pl.BlockSpec((D, H * Dh), lambda b, h: (0, 0)),
        ],
        out_specs=pl.BlockSpec((1, Sq, D), lambda b, h: (b, 0, 0)),
        out_shape=jax.ShapeDtypeStruct((B, Sq, D), x.dtype),
        scratch_shapes=[pltpu.VMEM((Sq, D), jnp.float32)],
        compiler_params=pltpu.CompilerParams(
            dimension_semantics=("arbitrary", "arbitrary"),
            vmem_limit_bytes=64 * 1024 * 1024,
        ),
    )(x, k_cache, v_cache, wq, wo.T)
```

```python
import jax
import jax.numpy as jnp
from jax import lax
import jax.experimental.pallas as pl
import jax.experimental.pallas.tpu as pltpu

_NT = (((1,), (1,)), ((), ()))
_F32 = jnp.float32

_NC = 8
_NB = 3
_QK_SPLIT = 3
_BODY_PTS = (16, 48, 64, 208, 80, 64, 80, 64, 80, 80, 64, 80, 64, 80, 64, 80, 64, 64, 16, 240)
_TAIL_PTS = (96, 96, 96, 160)
_SPIN = 20
_LEAD = 6


@jax.jit
def pallas_standalone__mha_block_cached__near_ridge_kernel(
    x: jax.Array,
    k_cache: jax.Array,
    v_cache: jax.Array,
    wq: jax.Array,
    wo: jax.Array,
):
    B, Sq, D = x.shape
    _, H, Sk, Dh = k_cache.shape
    dt = x.dtype
    scale = Dh ** -0.5
    N = B * H
    CK = Sk // _NC

    pts = list(_BODY_PTS) + list(_TAIL_PTS)
    assert sum(pts) == Sk
    J = len(pts) - _LEAD
    R0 = sum(pts[J:])
    offs = [R0 + sum(pts[:j]) if j < J else sum(pts[J:j]) for j in range(len(pts))]

    KB, VB = 0, _NB * Sk
    WQ = 2 * _NB * Sk
    WO = WQ + H * D
    ROWS = WO + H * D

    def kern(x_hbm, k_hbm, v_hbm, wq_hbm, wot_hbm, o_hbm,
             xbuf, big, s_ref, mp_ref, acc_ref, obuf, spin_ref, ksem, vsem, wsem, osem):
        def rows(base, n):
            return pl.ds(pl.multiple_of(base, 16), n)

        def kcopy(i, r0, n):
            slot = i % _NB
            return pltpu.make_async_copy(
                k_hbm.at[i, pl.ds(r0, n)], big.at[rows(KB + slot * Sk + r0, n)], ksem.at[slot])

        def vcopy(i):
            slot = i % _NB
            return pltpu.make_async_copy(
                v_hbm.at[i], big.at[rows(VB + slot * Sk, Sk)], vsem.at[slot])

        def out_head():
            return pltpu.make_async_copy(
                obuf.at[pl.ds(0, B - 1)], o_hbm.at[pl.ds(0, B - 1)], osem.at[0])

        def out_last():
            return pltpu.make_async_copy(obuf.at[B - 1], o_hbm.at[B - 1], osem.at[1])

        def qproj(i, pin):
            xb = xbuf[i // H]
            qs = []
            for t in range(Dh // 128):
                w = big[rows(WQ + (i % H) * D, D), t * 128:(t + 1) * 128]
                qs.append((jnp.dot(xb, w, preferred_element_type=_F32) * scale).astype(dt))
                pin()
            return jnp.concatenate(qs, axis=1)

        def qk_chunk(i, q, c, mp, pin):
            kc = big[rows(KB + (i % _NB) * Sk + c * CK, CK), :]
            s = lax.dot_general(q, kc, _NT, preferred_element_type=_F32)
            pin()
            s_ref[:, c * CK:(c + 1) * CK] = s
            for t in range(CK // 128):
                st = s[:, t * 128:(t + 1) * 128]
                mp = st if mp is None else jnp.maximum(mp, st)
            return mp

        def pv(i, m, pin):
            lp = None
            o = None
            for c in range(_NC):
                p = jnp.exp(s_ref[:, c * CK:(c + 1) * CK] - m)
                for t in range(CK // 128):
                    pt = p[:, t * 128:(t + 1) * 128]
                    lp = pt if lp is None else lp + pt
                vc = big[rows(VB + (i % _NB) * Sk + c * CK, CK), :]
                oc = jnp.dot(p.astype(dt), vc, preferred_element_type=_F32)
                pin()
                o = oc if o is None else o + oc
            l = jnp.sum(lp, axis=-1, keepdims=True)
            return (o / l).astype(dt)

        def oproj(i, o, pin):
            for r0, n in ((0, 256), (256, D - 256)):
                w = big[rows(WO + (i % H) * D + r0, n), :]
                y = lax.dot_general(o, w, _NT, preferred_element_type=_F32)
                pin()
                acc_ref[:, r0:r0 + n] += y

        def row_max():
            return jnp.max(mp_ref[...], axis=-1, keepdims=True)

        def nopin():
            pass

        xc = pltpu.make_async_copy(x_hbm, xbuf, wsem.at[0])
        xc.start()
        for h in range(H):
            pltpu.make_async_copy(wq_hbm.at[:, pl.ds(h * Dh, Dh)],
                                  big.at[pl.ds(WQ + h * D, D)], wsem.at[1]).start()
        kcopy(0, 0, Sk).start()
        for h in range(H):
            pltpu.make_async_copy(wot_hbm.at[:, pl.ds(h * Dh, Dh)],
                                  big.at[pl.ds(WO + h * D, D)], wsem.at[2]).start(priority=1)
        kcopy(1, 0, Sk).start(priority=1)
        kcopy(2, 0, R0).start(priority=1)
        vcopy(0).start(priority=1)
        vcopy(1).start(priority=1)
        acc_ref[...] = jnp.zeros_like(acc_ref)
        xc.wait()
        pltpu.make_async_copy(big.at[pl.ds(WQ, H * D)], big.at[pl.ds(WQ, H * D)], wsem.at[1]).wait()
        kcopy(0, 0, Sk).wait()

        q0 = qproj(0, nopin)
        mp0 = None
        for c in range(_NC):
            mp0 = qk_chunk(0, q0, c, mp0, nopin)
        mp_ref[...] = mp0
        pltpu.make_async_copy(big.at[pl.ds(WO, H * D)], big.at[pl.ds(WO, H * D)], wsem.at[2]).wait()

        def body(i, carry):
            cnt = [0]

            def pin():
                j = cnt[0]
                cnt[0] += 1
                tgt = i + 2 if j < J else i + 3

                @pl.when(tgt < N)
                def _():
                    kcopy(jnp.minimum(tgt, N - 1), offs[j], pts[j]).start(priority=0)

            @pl.when(i + 2 < N)
            def _():
                vcopy(jnp.minimum(i + 2, N - 1)).start(priority=1)

            kcopy(i + 1, 0, Sk).wait()
            vcopy(i).wait()

            m = row_max()
            q = qproj(i + 1, pin)
            o = pv(i, m, pin)
            mp = None
            for c in range(_QK_SPLIT):
                mp = qk_chunk(i + 1, q, c, mp, pin)
            oproj(i, o, pin)
            for c in range(_QK_SPLIT, _NC):
                mp = qk_chunk(i + 1, q, c, mp, pin)
            mp_ref[...] = mp

            @pl.when(i % H == H - 1)
            def _():
                obuf[i // H] = acc_ref[...].astype(dt)
                acc_ref[...] = jnp.zeros_like(acc_ref)

            def spin(t, c):
                spin_ref[0] = t
                return c

            for j in range(len(_TAIL_PTS)):
                if j:
                    lax.fori_loop(0, jnp.where(i + 3 < N, _SPIN, 0), spin, 0)
                pin()
            return carry

        lax.fori_loop(0, N - 1, body, 0)

        out_head().start()
        vcopy(N - 1).wait()
        o = pv(N - 1, row_max(), nopin)
        oproj(N - 1, o, nopin)
        obuf[B - 1] = acc_ref[...].astype(dt)
        out_last().start()
        out_head().wait()
        out_last().wait()

    any_spec = pl.BlockSpec(memory_space=pl.ANY)
    return pl.pallas_call(
        kern,
        in_specs=[any_spec] * 5,
        out_specs=any_spec,
        out_shape=jax.ShapeDtypeStruct((B, Sq, D), dt),
        scratch_shapes=[
            pltpu.VMEM((B, Sq, D), dt),
            pltpu.VMEM((ROWS, Dh), dt),
            pltpu.VMEM((Sq, Sk), _F32),
            pltpu.VMEM((Sq, 128), _F32),
            pltpu.VMEM((Sq, D), _F32),
            pltpu.VMEM((B, Sq, D), dt),
            pltpu.SMEM((1,), jnp.int32),
            pltpu.SemaphoreType.DMA((_NB,)),
            pltpu.SemaphoreType.DMA((_NB,)),
            pltpu.SemaphoreType.DMA((3,)),
            pltpu.SemaphoreType.DMA((2,)),
        ],
        compiler_params=pltpu.CompilerParams(
            vmem_limit_bytes=64 * 1024 * 1024,
            disable_bounds_checks=True,
        ),
    )(x, k_cache.reshape(N, Sk, Dh), v_cache.reshape(N, Sk, Dh), wq, wo.T)
```

```python
import jax
import jax.numpy as jnp
from jax import lax
import jax.experimental.pallas as pl
import jax.experimental.pallas.tpu as pltpu

_NT = (((1,), (1,)), ((), ()))
_F32 = jnp.float32

_NC = 8
_NB = 3
_PR = 96
_KOFF = 16
_QK_SPLIT = 3
_NTAIL = 4
_SPIN = (20, 20, 20, 19)
_LEAD = 7
_ENDCUT = 2
_PRO_SPIN = 26

_PLAN = {1: [(0, 0)], 2: ["F"], 3: [(1, 16), (1, 104)], 19: [(18, 112)]}
for _g in (4, 8, 12, 16):
    _PLAN.update({_g: [None], _g + 1: [(_g, 24)], _g + 2: [(_g + 1, 72)]})
_PRO_PLAN = {3: [(0, 0), (1, 96)], 5: [None], 6: [(5, 72)], 8: [(7, 24)], 10: [None], 11: [(10, 96)]}


@jax.jit
def pallas_standalone__mha_block_cached__near_ridge_kernel(
    x: jax.Array,
    k_cache: jax.Array,
    v_cache: jax.Array,
    wq: jax.Array,
    wo: jax.Array,
):
    B, Sq, D = x.shape
    _, H, Sk, Dh = k_cache.shape
    dt = x.dtype
    scale = Dh ** -0.5
    N = B * H
    L = N - 1
    CK = Sk // _NC

    nbody = 1 + sum(p != "F" for v in _PLAN.values() for p in v)
    NP = nbody + _NTAIL
    J = NP - _LEAD
    pts = [_PR] * NP
    pts[J] += _KOFF
    pts[J - 1] += Sk - sum(pts)
    R0 = sum(pts[J:])
    offs = [R0 + sum(pts[:j]) if j < J else sum(pts[J:j]) for j in range(NP)]
    assert sum(len(v) for v in _PRO_PLAN.values()) == _LEAD
    RT = offs[J - _ENDCUT]
    avail = [c for c in range(_NC) if c * CK >= R0 and (c + 1) * CK <= RT]
    late = [c for c in range(_NC) if c not in avail]
    NK = Sk // _PR
    KEND = _KOFF + NK * _PR

    KB, VB = 0, _NB * Sk
    MARK = 2 * _NB * Sk
    ROWS = MARK + 16
    XR = Sq // 3
    OCOLS = ((0, 256), (256, D - 256))

    def kern(x_hbm, k_hbm, v_hbm, wq_hbm, wot_hbm, o_hbm,
             xbuf, big, wqbuf, wobuf, s_ref, s2_ref, mp_ref, ql_ref, acc_ref, obuf, spin_ref,
             ksem, vsem, wsem, osem):
        def rows(base, n, align=16):
            if isinstance(base, int):
                return pl.ds(base, n)
            return pl.ds(pl.multiple_of(base, align), n)

        def cols(h, c0, n):
            return rows(h * Dh + c0, n, 128)

        def kcopy(i, slot, r0, n, sem=None):
            return pltpu.make_async_copy(
                k_hbm.at[i, rows(r0, n)], big.at[rows(KB + slot * Sk + r0, n)],
                ksem.at[slot] if sem is None else sem)

        def vcopy(i, slot, r0=0, n=Sk):
            return pltpu.make_async_copy(
                v_hbm.at[i, rows(r0, n)], big.at[rows(VB + slot * Sk + r0, n)], vsem.at[slot])

        def out_head():
            return pltpu.make_async_copy(
                obuf.at[pl.ds(0, B - 1)], o_hbm.at[pl.ds(0, B - 1)], osem.at[0])

        def out_last(t):
            c = pl.ds(*OCOLS[t])
            return pltpu.make_async_copy(obuf.at[B - 1, :, c], o_hbm.at[B - 1, :, c], osem.at[1 + t])

        def spin(n):
            def step(t, c):
                spin_ref[0] = t
                return c
            lax.fori_loop(0, n, step, 0)

        def pinner(plan, inject):
            res = []

            def pin(r):
                res.append(r)
                for p in plan.get(len(res) - 1, ()):
                    if p == "F":
                        big[pl.ds(MARK, 8), 0:128] = jnp.zeros((8, 128), dt)
                        continue
                    if p is not None:
                        big[pl.ds(MARK, 8), 0:128] = res[p[0]][p[1]:p[1] + 8, 0:128].astype(dt)
                    inject()
            return pin

        def nopin(_):
            pass

        def qproj(b, h, pin):
            xb = xbuf[b]
            qs = []
            for t in range(Dh // 128):
                qt = jnp.dot(xb, wqbuf[:, cols(h, t * 128, 128)], preferred_element_type=_F32)
                qs.append((qt * scale).astype(dt))
                pin(qt)
            return jnp.concatenate(qs, axis=1)

        def qk_chunk(slot, q, c, mp, pin, sref):
            kc = big[rows(KB + slot * Sk + c * CK, CK, CK), :]
            s = lax.dot_general(q, kc, _NT, preferred_element_type=_F32)
            pin(s)
            sref[:, c * CK:(c + 1) * CK] = s
            for t in range(CK // 128):
                st = s[:, t * 128:(t + 1) * 128]
                mp = st if mp is None else jnp.maximum(mp, st)
            return mp

        def pv(slot, m, pin, sref, zero=None):
            lp = None
            o = None
            ocs = []
            for c in range(_NC):
                if zero is not None and c >= 2:
                    sref[rows(zero, 8, 8), (c - 2) * CK:(c - 2) * CK + 128] = ocs[c - 2][0:8, 0:128]
                p = jnp.exp(sref[:, c * CK:(c + 1) * CK] - m)
                for t in range(CK // 128):
                    pt = p[:, t * 128:(t + 1) * 128]
                    lp = pt if lp is None else lp + pt
                vc = big[rows(VB + slot * Sk + c * CK, CK, CK), :]
                oc = jnp.dot(p.astype(dt), vc, preferred_element_type=_F32)
                pin(oc)
                ocs.append(oc)
                o = oc if o is None else o + oc
            l = jnp.sum(lp, axis=-1, keepdims=True)
            return (o / l).astype(dt)

        def oproj_part(h, o, t):
            r0, n = OCOLS[t]
            return lax.dot_general(o, wobuf[r0:r0 + n, cols(h, 0, Dh)], _NT,
                                   preferred_element_type=_F32)

        def oproj(h, o, pin):
            for t, (r0, n) in enumerate(OCOLS):
                y = oproj_part(h, o, t)
                pin(y)
                acc_ref[:, r0:r0 + n] += y

        def paced(n, mk):
            def step(j, c):
                mk(j).start(priority=0)
                spin(_PRO_SPIN)
                return c
            lax.fori_loop(0, n, step, 0)

        pltpu.make_async_copy(wq_hbm, wqbuf, wsem.at[1]).start(priority=1)
        paced(NK, lambda j: kcopy(0, 0, _KOFF + j * _PR, _PR))
        pltpu.make_async_copy(wot_hbm, wobuf, wsem.at[2]).start(priority=1)
        for copy, i in ((kcopy, 0), (kcopy, 1), (vcopy, 0)):
            copy(i, i, 0, _KOFF).start(priority=0)
            copy(i, i, KEND, Sk - KEND).start(priority=0)
        spin(_PRO_SPIN)
        vcopy(1, 1).start(priority=1)

        def x_step(j, c):
            for t in range(Sq // XR):
                r = pl.ds(t * XR, XR)
                pltpu.make_async_copy(x_hbm.at[j, r], xbuf.at[j, r], wsem.at[0]).start(priority=0)
                spin(_PRO_SPIN)
            return c
        lax.fori_loop(0, B, x_step, 0)
        paced(NK, lambda j: kcopy(1, 1, _KOFF + j * _PR, _PR))
        paced(NK, lambda j: vcopy(0, 0, _KOFF + j * _PR, _PR))

        pltpu.make_async_copy(x_hbm, xbuf, wsem.at[0]).wait()
        pltpu.make_async_copy(wq_hbm, wqbuf, wsem.at[1]).wait()
        kcopy(0, 0, 0, Sk).wait()

        pro_cnt = [J]

        def pro_inject():
            kcopy(2, 2, offs[pro_cnt[0]], pts[pro_cnt[0]]).start(priority=0)
            pro_cnt[0] += 1

        pro_pin = pinner(_PRO_PLAN, pro_inject)
        acc_ref[...] = jnp.zeros_like(acc_ref)
        q0 = qproj(0, 0, pro_pin)
        ql_ref[...] = qproj(L // H, L % H, pro_pin)
        mp0 = None
        for c in range(_NC):
            mp0 = qk_chunk(0, q0, c, mp0, pro_pin, s_ref)
        mp_ref[...] = mp0
        pltpu.make_async_copy(wot_hbm, wobuf, wsem.at[2]).wait()

        def body(i, carry):
            s0 = lax.rem(i, _NB)
            s1 = lax.rem(i + 1, _NB)
            s2 = lax.rem(i + 2, _NB)
            h = lax.rem(i, H)
            hn = lax.rem(i + 1, H)
            bn = lax.div(i + 1, H)
            early = i + 3 < L
            i3 = jnp.minimum(i + 3, L)
            cnt = [0]

            def inject():
                j = cnt[0]
                cnt[0] += 1
                if j < J - _ENDCUT:
                    kcopy(i + 2, s2, offs[j], pts[j]).start(priority=0)
                    if j == 4:
                        @pl.when(i + 3 == L)
                        def _():
                            kcopy(i + 2, s2, RT, Sk - RT).start(priority=0)
                else:
                    @pl.when(early)
                    def _():
                        if j < J:
                            kcopy(i + 2, s2, offs[j], pts[j]).start(priority=0)
                        else:
                            kcopy(i3, s0, offs[j], pts[j]).start(priority=0)

            pin = pinner(_PLAN, inject)

            vcopy(i + 2, s2).start(priority=1)
            vcopy(i, s0).wait()
            inject()
            kcopy(i + 1, s1, 0, Sk).wait()

            m = jnp.max(mp_ref[...], axis=-1, keepdims=True)
            q = qproj(bn, hn, pin)
            o = pv(s0, m, pin, s_ref)
            mp = None
            for c in range(_QK_SPLIT):
                mp = qk_chunk(s1, q, c, mp, pin, s_ref)
            oproj(h, o, pin)
            for c in range(_QK_SPLIT, _NC):
                mp = qk_chunk(s1, q, c, mp, pin, s_ref)
            mp_ref[...] = mp

            @pl.when(hn == 0)
            def _():
                obuf[bn - 1] = acc_ref[...].astype(dt)
                acc_ref[...] = jnp.zeros_like(acc_ref)

            @pl.when(early)
            def _():
                for j in range(_NTAIL):
                    kcopy(i3, s0, offs[nbody + j], pts[nbody + j]).start(priority=0)
                    spin(_SPIN[j])

            return lax.shift_right_logical(i, 16)

        zero = lax.fori_loop(0, N - 2, body, jnp.int32(0))
        zero = jnp.clip(zero, 0, Sq // 8 - 1) * 8

        sa, sl = (L - 1) % _NB, L % _NB
        vcopy(L - 1, sa).wait()
        kcopy(L, sl, 0, R0, wsem.at[3]).start(priority=0)
        kcopy(L, sl, RT, Sk - RT, wsem.at[3]).start(priority=0)
        kcopy(L, sl, R0, RT - R0).wait()

        m = jnp.max(mp_ref[...], axis=-1, keepdims=True)
        q = ql_ref[...]
        mp = None
        for c in avail[:2]:
            mp = qk_chunk(sl, q, c, mp, nopin, s2_ref)
        o1 = pv(sa, m, nopin, s_ref, zero)
        for c in avail[2:]:
            mp = qk_chunk(sl, q, c, mp, nopin, s2_ref)

        kcopy(L, sl, 0, R0, wsem.at[3]).wait()
        kcopy(L, sl, RT, Sk - RT, wsem.at[3]).wait()
        res = []
        for c in late:
            mp = qk_chunk(sl, q, c, mp, res.append, s2_ref)
        obuf[B - 1, 0:8, 0:128] = res[1][64:72, 0:128].astype(dt)
        out_head().start()

        vcopy(L, sl).wait()
        m = jnp.max(mp, axis=-1, keepdims=True)
        oproj((L - 1) % H, o1, nopin)
        o2 = pv(sl, m, nopin, s2_ref, zero)
        for t, (r0, n) in enumerate(OCOLS):
            obuf[B - 1, :, r0:r0 + n] = (acc_ref[:, r0:r0 + n] + oproj_part(L % H, o2, t)).astype(dt)
            out_last(t).start()
        out_head().wait()
        for t in range(len(OCOLS)):
            out_last(t).wait()

    any_spec = pl.BlockSpec(memory_space=pl.ANY)
    return pl.pallas_call(
        kern,
        in_specs=[any_spec] * 5,
        out_specs=any_spec,
        out_shape=jax.ShapeDtypeStruct((B, Sq, D), dt),
        scratch_shapes=[
            pltpu.VMEM((B, Sq, D), dt),
            pltpu.VMEM((ROWS, Dh), dt),
            pltpu.VMEM((D, H * Dh), dt),
            pltpu.VMEM((D, H * Dh), dt),
            pltpu.VMEM((Sq, Sk), _F32),
            pltpu.VMEM((Sq, Sk), _F32),
            pltpu.VMEM((Sq, 128), _F32),
            pltpu.VMEM((Sq, Dh), dt),
            pltpu.VMEM((Sq, D), _F32),
            pltpu.VMEM((B, Sq, D), dt),
            pltpu.SMEM((1,), jnp.int32),
            pltpu.SemaphoreType.DMA((_NB,)),
            pltpu.SemaphoreType.DMA((_NB,)),
            pltpu.SemaphoreType.DMA((4,)),
            pltpu.SemaphoreType.DMA((3,)),
        ],
        compiler_params=pltpu.CompilerParams(
            vmem_limit_bytes=64 * 1024 * 1024,
            disable_bounds_checks=True,
            disable_semaphore_checks=True,
        ),
    )(x, k_cache.reshape(N, Sk, Dh), v_cache.reshape(N, Sk, Dh), wq, wo.T)
```
